```python
import jax
import jax.numpy as jnp

def _softmax(x, axis=-1):
    return jax.nn.softmax(x, axis=axis)
def _gelu(x):
    return jax.nn.gelu(x, approximate=True)
def _silu(x):
    return jax.nn.silu(x)
def _sigmoid(x):
    return jax.nn.sigmoid(x)
def _layernorm(x, axis=-1, eps=1e-5):
    m = jnp.mean(x, axis=axis, keepdims=True)
    v = jnp.var(x, axis=axis, keepdims=True)
    return (x - m) / jnp.sqrt(v + eps)
def _scatter_add(tgt, idx, src, axis=0):
    return tgt.at[idx].add(src)
def _segment_sum(src, seg, n):
    return jax.ops.segment_sum(src, seg, n)
class _Rng:
    def __init__(self, key):
        self._k = key
    def _next(self):
        self._k, sub = jax.random.split(self._k)
        return sub
    def normal(self, shape):
        return jax.random.normal(self._next(), shape, dtype=jnp.bfloat16)
    def randint(self, lo, hi, shape):
        return jax.random.randint(self._next(), shape, lo, hi, dtype=jnp.int32)
    def uniform(self, shape, lo=0.0, hi=1.0):
        return jax.random.uniform(self._next(), shape, jnp.bfloat16, lo, hi)
    def permutation(self, n):
        return jax.random.permutation(self._next(), n)


kernel_name = 'recurrent_scan__gqa_block_cached__geglu_ffn__decode'

def _fwd_setup_inputs():
    _rng = _Rng(jax.random.key(int.from_bytes(__import__("os").urandom(4), "little")))
    _w = (lambda a: (lambda t: t.astype(jnp.bfloat16) if jnp.issubdtype(t.dtype, jnp.floating) else t)(jnp.asarray(a)))
    def _A_setup():
        B, Sq, D = 1, 1, 512
        Hq, Hkv, Sk, Dh = 32, 32, 4096, 128
        assert Hq % Hkv == 0, (Hq, Hkv)
        return {
            "x": _w((lambda *s: _rng.normal(s) * 0.05)(B, Sq, D)),
            "k_cache": _w((lambda *s: _rng.normal(s) * 0.05)(B, Hkv, Sk, Dh)),
            "v_cache": _w((lambda *s: _rng.normal(s) * 0.05)(B, Hkv, Sk, Dh)),
            "wq": _w((lambda *s: _rng.normal(s) * 0.05)(D, Hq * Dh) * (D ** -0.5)),
            "wo": _w((lambda *s: _rng.normal(s) * 0.05)(Hq * Dh, D) * ((Hq * Dh) ** -0.5)),
        }
    _A_in = _A_setup()

    def _B_setup():
        B, S, D, F = 1, 1, 512, 1376
        return {
            "x": _w((lambda *s: _rng.normal(s) * 0.05)(B, S, D)),
            "w_gate": _w((lambda *s: _rng.normal(s) * 0.05)(D, F)),
            "w_up": _w((lambda *s: _rng.normal(s) * 0.05)(D, F)),
            "w_down": _w((lambda *s: _rng.normal(s) * 0.05)(F, D)),
        }
    _B_in = _B_setup()

    return {
        "A_x": _A_in["x"],
        "A_k_cache": _A_in["k_cache"],
        "A_v_cache": _A_in["v_cache"],
        "A_wq": _A_in["wq"],
        "A_wo": _A_in["wo"],
        "B_x": _B_in["x"],
        "B_w_gate": _B_in["w_gate"],
        "B_w_up": _B_in["w_up"],
        "B_w_down": _B_in["w_down"],
    }

def _fwd_reference(A_x, A_k_cache, A_v_cache, A_wq, A_wo, B_x, B_w_gate, B_w_up, B_w_down):
    def _A_ref(x, k_cache, v_cache, wq, wo):
        B, Sq, D = x.shape
        Hq, Dh = 32, 128
        Hkv = k_cache.shape[1]
        rep = Hq // Hkv
        q = (lambda x, *d: x.transpose(*d))((x @ wq).reshape(B, Sq, Hq, Dh), 0, 2, 1, 3)
        k = jnp.repeat(k_cache, rep, axis=1)
        v = jnp.repeat(v_cache, rep, axis=1)
        scores = jnp.einsum("bhqd,bhkd->bhqk", q, k) * (Dh ** -0.5)
        p = _softmax(scores, axis=-1)
        o = jnp.einsum("bhqk,bhkd->bhqd", p, v)
        return (lambda x, *d: x.transpose(*d))(o, 0, 2, 1, 3).reshape(B, Sq, Hq * Dh) @ wo

    def _B_ref(x, w_gate, w_up, w_down):
        return (_gelu(x @ w_gate) * (x @ w_up)) @ w_down

    x = A_x
    xn = _layernorm(x, axis=-1)
    s = _A_ref(xn, A_k_cache, A_v_cache, A_wq, A_wo)
    g = _silu(_B_ref(xn, B_w_gate, B_w_up, B_w_down))
    return x + s * g


def setup_inputs():
    _inp = _fwd_setup_inputs()
    _gk = jax.random.fold_in(jax.random.key(int.from_bytes(__import__("os").urandom(4), "little")), 2**31 - 1)
    _shapes = [[1, 1, 512]]
    _dtypes = ['bfloat16']
    _gks = jax.random.split(_gk, len(_shapes))
    _gs = [jax.random.normal(k, s, dtype=jnp.dtype(d)) * 0.05 for k, s, d in zip(_gks, _shapes, _dtypes)]
    _inp["grad_out"] = _gs[0]
    return _inp

def reference(A_x, A_k_cache, A_v_cache, A_wq, A_wo, B_w_gate, B_w_up, B_w_down, B_x, grad_out):
    _const = dict(B_x=B_x)
    def _f(*_d):
        return _fwd_reference(**{'A_x': _d[0], 'A_k_cache': _d[1], 'A_v_cache': _d[2], 'A_wq': _d[3], 'A_wo': _d[4], 'B_w_gate': _d[5], 'B_w_up': _d[6], 'B_w_down': _d[7], **_const})
    _out, _vjp = jax.vjp(_f, A_x, A_k_cache, A_v_cache, A_wq, A_wo, B_w_gate, B_w_up, B_w_down)
    _grads = _vjp(grad_out)
    _out0 = jnp.asarray(_out)
    return (_out0, *[jnp.asarray(_g) for _g in _grads])
```

```python
import math

import jax
import jax.numpy as jnp
from jax import lax
import jax.experimental.pallas as pl
import jax.experimental.pallas.tpu as pltpu

F32 = jnp.float32
BF16 = jnp.bfloat16
LANES = 128
SUBLANES = 8
HEAD_DIM = 128
LN_EPS = 1e-5
GELU_C = math.sqrt(2.0 / math.pi)
GELU_A = 0.044715

HEADS_PER_WRITE = 8
ROWS_PER_WRITE = 64
TAIL_ROWS = 1024


def _nn(a, b):
    return jnp.dot(a.astype(BF16), b, preferred_element_type=F32)


def _nt(a, b):
    return lax.dot_general(
        a.astype(BF16), b, (((1,), (1,)), ((), ())), preferred_element_type=F32
    )


def _column(row):
    return jnp.broadcast_to(row, (LANES, LANES)).T


def _store_outer(out_ref, left, right):
    n = left.shape[1]
    for start in range(0, n, LANES):
        start = min(start, n - LANES)
        col = _column(left[0:1, start:start + LANES])
        for j in range(0, right.shape[1], LANES):
            blk = col * right[0:1, j:j + LANES]
            out_ref[start:start + LANES, j:j + LANES] = blk.astype(out_ref.dtype)


def _store_outer_tall(out_ref, left, right):
    col = _column(right[0:1])
    for i in range(0, left.shape[1], LANES):
        blk = (col * left[0:1, i:i + LANES]).astype(out_ref.dtype)
        out_ref[i:i + LANES, :] = blk.T


def _kernel(
    x_hbm, k_hbm, v_hbm, wq_hbm, wo_hbm, wg_hbm, wu_hbm, wd_hbm, dy_hbm,
    y_hbm, dx_hbm, dk_hbm, dv_hbm, dwq_hbm, dwo_hbm, dwg_hbm, dwu_hbm, dwd_hbm,
    x_buf, dy_buf, k_buf, v_buf, wq_buf, wo_buf, wg_buf, wu_buf, wd_buf,
    q_scr, do_scr, o_scr, dq_scr,
    head_sems, sems,
):
    heads, seq, _ = k_buf.shape
    d_model = x_buf.shape[-1]
    scale = HEAD_DIM ** -0.5
    last = heads - 1
    copy = pltpu.make_async_copy

    def head_reads(h):
        return (
            copy(k_hbm.at[0, h], k_buf.at[h], head_sems.at[h]),
            copy(v_hbm.at[0, h], v_buf.at[h], head_sems.at[h]),
        )

    first_reads = [
        copy(wq_hbm, wq_buf, sems.at[0]),
        copy(x_hbm, x_buf, sems.at[0]),
        copy(dy_hbm, dy_buf, sems.at[0]),
    ]
    weight_reads = [
        copy(wg_hbm, wg_buf, sems.at[1]),
        copy(wu_hbm, wu_buf, sems.at[1]),
        copy(wd_hbm, wd_buf, sems.at[1]),
        copy(wo_hbm, wo_buf, sems.at[1]),
    ]
    body_rows = pl.ds(0, seq - TAIL_ROWS)
    tail_rows = pl.ds(seq - TAIL_ROWS, TAIL_ROWS)
    last_reads = [
        copy(k_hbm.at[0, last], k_buf.at[last], head_sems.at[last]),
        copy(v_hbm.at[0, last, body_rows], v_buf.at[last, body_rows], head_sems.at[last]),
    ]
    tail_read = copy(v_hbm.at[0, last, tail_rows], v_buf.at[last, tail_rows], sems.at[2])

    for c in first_reads + weight_reads:
        c.start()

    @pl.loop(0, last)
    def _(h):
        for c in head_reads(h):
            c.start()

    for c in last_reads + [tail_read]:
        c.start()

    for c in first_reads:
        c.wait()
    x = jnp.broadcast_to(x_buf[0].astype(F32), (SUBLANES, d_model))
    dy = jnp.broadcast_to(dy_buf[0].astype(F32), (SUBLANES, d_model))
    xc = x - jnp.mean(x, axis=-1, keepdims=True)
    rstd = lax.rsqrt(jnp.mean(xc * xc, axis=-1, keepdims=True) + LN_EPS)
    xn = xc * rstd
    q = _nn(xn, wq_buf[...])
    for h in range(heads):
        q_scr[h] = q[:, h * HEAD_DIM:(h + 1) * HEAD_DIM]

    for c in weight_reads:
        c.wait()
    a = _nt(xn, wg_buf[...])
    u = _nt(xn, wu_buf[...])
    t = jnp.tanh(GELU_C * (a + GELU_A * a * a * a))
    act = 0.5 * a * (1.0 + t)
    mid = act * u
    f = _nn(mid, wd_buf[...])
    sig = jax.nn.sigmoid(f)
    gate = f * sig
    d_attn = dy * gate
    do = _nt(d_attn, wo_buf[...])
    for h in range(heads):
        do_scr[h] = do[:, h * HEAD_DIM:(h + 1) * HEAD_DIM]

    def attend(h):
        k_ref, v_ref = k_buf.at[h], v_buf.at[h]
        q_h, do_h = q_scr[h], do_scr[h]
        s = _nt(q_h, k_ref[...]) * scale
        dp = _nt(do_h, v_ref[...])
        e = jnp.exp(s - jnp.max(s, axis=-1, keepdims=True))
        p = e * (1.0 / jnp.sum(e, axis=-1, keepdims=True))
        ds = p * (dp - jnp.sum(p * dp, axis=-1, keepdims=True)) * scale
        o_scr[h] = _nn(p, v_ref[...])
        dq_scr[h] = _nn(ds, k_ref[...])
        _store_outer_tall(v_ref, p, do_h)
        _store_outer_tall(k_ref, ds, q_h)

    @pl.loop(0, last)
    def _(h):
        for c in head_reads(h):
            c.wait()
        attend(h)

    def start_cache_writes(buf, hbm, group):
        hs = pl.ds(group * HEADS_PER_WRITE, HEADS_PER_WRITE)

        @pl.loop(0, seq // ROWS_PER_WRITE)
        def _(j):
            rows = pl.ds(pl.multiple_of(j * ROWS_PER_WRITE, ROWS_PER_WRITE), ROWS_PER_WRITE)
            copy(buf.at[hs, rows], hbm.at[0, hs, rows], sems.at[3]).start()

    for c in last_reads:
        c.wait()
    start_cache_writes(k_buf, dk_hbm, 0)
    tail_read.wait()
    attend(last)
    start_cache_writes(v_buf, dv_hbm, 0)

    o = jnp.concatenate([o_scr[h] for h in range(heads)], axis=1)
    dq = jnp.concatenate([dq_scr[h] for h in range(heads)], axis=1)
    attn = _nn(o, wo_buf[...])
    df = dy * attn * (sig + gate * (1.0 - sig))
    dmid = _nt(df, wd_buf[...])
    dact = 0.5 * (1.0 + t) + 0.5 * a * (1.0 - t * t) * GELU_C * (1.0 + 3.0 * GELU_A * a * a)
    da = dmid * u * dact
    du = dmid * act
    dxn = _nt(dq, wq_buf[...]) + _nn(da, wg_buf[...]) + _nn(du, wu_buf[...])
    dx = dy + rstd * (
        dxn
        - jnp.mean(dxn, axis=-1, keepdims=True)
        - xn * jnp.mean(dxn * xn, axis=-1, keepdims=True)
    )
    x_buf[0] = (x + attn * gate)[0:1].astype(BF16)
    dy_buf[0] = dx[0:1].astype(BF16)
    start_cache_writes(k_buf, dk_hbm, 1)

    _store_outer(wq_buf, xn, dq)
    _store_outer(wo_buf, o, d_attn)
    start_cache_writes(v_buf, dv_hbm, 1)
    _store_outer(wg_buf, da, xn)
    _store_outer(wu_buf, du, xn)
    _store_outer(wd_buf, mid, df)

    small_writes = [
        copy(x_buf, y_hbm, sems.at[3]),
        copy(dy_buf, dx_hbm, sems.at[3]),
        copy(wq_buf, dwq_hbm, sems.at[3]),
        copy(wo_buf, dwo_hbm, sems.at[3]),
        copy(wg_buf, dwg_hbm, sems.at[3]),
        copy(wu_buf, dwu_hbm, sems.at[3]),
        copy(wd_buf, dwd_hbm, sems.at[3]),
    ]
    for c in small_writes:
        c.start()
    for group in range(2, heads // HEADS_PER_WRITE):
        start_cache_writes(k_buf, dk_hbm, group)
        start_cache_writes(v_buf, dv_hbm, group)

    for c in small_writes:
        c.wait()
    copy(k_buf, dk_hbm.at[0], sems.at[3]).wait()
    copy(v_buf, dv_hbm.at[0], sems.at[3]).wait()


@jax.jit
def pallas_recurrent_scan__gqa_block_cached__geglu_ffn__decode_kernel(
    A_x: jax.Array,
    A_k_cache: jax.Array,
    A_v_cache: jax.Array,
    A_wq: jax.Array,
    A_wo: jax.Array,
    B_x: jax.Array,
    B_w_gate: jax.Array,
    B_w_up: jax.Array,
    B_w_down: jax.Array,
    grad_out: jax.Array,
):
    del B_x
    _, heads, seq, head_dim = A_k_cache.shape
    w_gate_t, w_up_t = B_w_gate.T, B_w_up.T
    operands = (A_x, A_k_cache, A_v_cache, A_wq, A_wo, w_gate_t, w_up_t, B_w_down, grad_out)
    results = (A_x, A_x, A_k_cache, A_v_cache, A_wq, A_wo, w_gate_t, w_up_t, B_w_down)
    hbm = pl.BlockSpec(memory_space=pltpu.HBM)
    per_head = pltpu.VMEM((heads, SUBLANES, head_dim), F32)

    y, dx, dk, dv, dwq, dwo, dwg_t, dwu_t, dwd = pl.pallas_call(
        _kernel,
        in_specs=[hbm] * len(operands),
        out_specs=[hbm] * len(results),
        out_shape=[jax.ShapeDtypeStruct(r.shape, r.dtype) for r in results],
        scratch_shapes=[
            pltpu.VMEM(A_x.shape, BF16),
            pltpu.VMEM(grad_out.shape, BF16),
            pltpu.VMEM((heads, seq, head_dim), BF16),
            pltpu.VMEM((heads, seq, head_dim), BF16),
            pltpu.VMEM(A_wq.shape, BF16),
            pltpu.VMEM(A_wo.shape, BF16),
            pltpu.VMEM(w_gate_t.shape, BF16),
            pltpu.VMEM(w_up_t.shape, BF16),
            pltpu.VMEM(B_w_down.shape, BF16),
            per_head,
            per_head,
            per_head,
            per_head,
            pltpu.SemaphoreType.DMA((heads,)),
            pltpu.SemaphoreType.DMA((4,)),
        ],
        compiler_params=pltpu.CompilerParams(vmem_limit_bytes=100 * 1024 * 1024),
    )(*operands)
    return y, dx, dk, dv, dwq, dwo, dwg_t.T, dwu_t.T, dwd
```

```python
import math

import jax
import jax.numpy as jnp
from jax import lax
import jax.experimental.pallas as pl
import jax.experimental.pallas.tpu as pltpu

F32 = jnp.float32
BF16 = jnp.bfloat16
LANES = 128
SUBLANES = 8
LN_EPS = 1e-5
GELU_C = math.sqrt(2.0 / math.pi)
GELU_A = 0.044715

WRITE_HEADS = 8
WRITE_ROWS = 16
READ_TAIL_ROWS = 1792


def _matmul(a, b):
    return jnp.dot(a.astype(BF16), b, preferred_element_type=F32)


def _matmul_t(a, b):
    return lax.dot_general(
        a.astype(BF16), b, (((1,), (1,)), ((), ())), preferred_element_type=F32
    )


def _mean(v):
    return jnp.mean(v, axis=-1, keepdims=True)


def _block(index, size):
    return pl.ds(pl.multiple_of(index * size, size), size)


def _column(row):
    return jnp.broadcast_to(row, (LANES, LANES)).T


def _store_outer(out_ref, left, right):
    n = left.shape[1]
    for i in range(0, n, LANES):
        i = min(i, n - LANES)
        col = _column(left[0:1, i:i + LANES])
        for j in range(0, right.shape[1], LANES):
            tile = col * right[0:1, j:j + LANES]
            out_ref[i:i + LANES, j:j + LANES] = tile.astype(out_ref.dtype)


def _store_tall_outer(out_ref, left, right):
    col = _column(right[0:1])
    for i in range(0, left.shape[1], LANES):
        tile = col * left[0:1, i:i + LANES]
        out_ref[i:i + LANES, :] = tile.astype(out_ref.dtype).T


def _kernel(
    x_hbm, k_hbm, v_hbm, wq_hbm, wo_hbm, wg_hbm, wu_hbm, wd_hbm, dy_hbm,
    y_hbm, dx_hbm, dk_hbm, dv_hbm, dwq_hbm, dwo_hbm, dwg_hbm, dwu_hbm, dwd_hbm,
    x_buf, dy_buf, k_buf, v_buf, wq_buf, wo_buf, wg_buf, wu_buf, wd_buf,
    xn_col, write_sem,
):
    heads, seq, head_dim = k_buf.shape
    d_model = x_buf.shape[-1]
    scale = head_dim ** -0.5
    last = heads - 1
    copy = pltpu.make_async_copy

    def write_cache(buf, hbm, group):
        hs = pl.ds(group * WRITE_HEADS, WRITE_HEADS)

        @pl.loop(0, seq // WRITE_ROWS, unroll=4)
        def _(j):
            rows = _block(j, WRITE_ROWS)
            copy(buf.at[hs, rows], hbm.at[0, hs, rows], write_sem).start()

    def write_weights(pairs, regions, rows, cols):
        n_rows, n_cols = pairs[0][0].shape
        shape = (regions, n_rows // regions, n_cols)

        @pl.loop(0, shape[1] // rows)
        def _(j):
            for c in range(0, n_cols, cols):
                idx = (slice(None), _block(j, rows), pl.ds(c, cols))
                for buf, hbm in pairs:
                    src, dst = buf.reshape(shape), hbm.reshape(shape)
                    copy(src.at[idx], dst.at[idx], write_sem).start()

    def read_and_compute(head_sems, sems):
        ffn_reads = [
            copy(hbm, buf, sems.at[0])
            for hbm, buf in (
                (wg_hbm, wg_buf), (x_hbm, x_buf), (dy_hbm, dy_buf),
                (wu_hbm, wu_buf), (wd_hbm, wd_buf),
            )
        ]
        projection_reads = [
            copy(wq_hbm, wq_buf, sems.at[1]),
            copy(wo_hbm, wo_buf, sems.at[1]),
        ]
        body = pl.ds(0, seq - READ_TAIL_ROWS)
        tail = pl.ds(seq - READ_TAIL_ROWS, READ_TAIL_ROWS)
        tail_read = copy(v_hbm.at[0, last, tail], v_buf.at[last, tail], sems.at[2])

        def k_read(h):
            return copy(k_hbm.at[0, h], k_buf.at[h], head_sems.at[h])

        def v_read(h, rows=slice(None)):
            return copy(v_hbm.at[0, h, rows], v_buf.at[h, rows], head_sems.at[h])

        for c in ffn_reads + projection_reads:
            c.start()

        @pl.loop(0, last)
        def _(h):
            k_read(h).start()
            v_read(h).start()

        k_read(last).start()
        v_read(last, body).start()
        tail_read.start()

        for c in ffn_reads:
            c.wait()
        x = jnp.broadcast_to(x_buf[0].astype(F32), (SUBLANES, d_model))
        dy = jnp.broadcast_to(dy_buf[0].astype(F32), (SUBLANES, d_model))
        centred = x - _mean(x)
        rstd = lax.rsqrt(_mean(centred * centred) + LN_EPS)
        xn = centred * rstd
        for i in range(0, d_model, LANES):
            xn_col[i:i + LANES, :] = _column(xn[0:1, i:i + LANES])

        a = _matmul_t(xn, wg_buf[...])
        u = _matmul_t(xn, wu_buf[...])
        t = jnp.tanh(GELU_C * (a + GELU_A * a * a * a))
        act = 0.5 * a * (1.0 + t)
        mid = act * u
        f = _matmul(mid, wd_buf[...])
        sig = jax.nn.sigmoid(f)
        gate = f * sig
        d_attn = dy * gate

        for c in projection_reads:
            c.wait()

        def head(h, carry):
            k_read(h).wait()

            @pl.when(h < last)
            def _():
                v_read(h).wait()

            @pl.when(h == last)
            def _():
                v_read(last, body).wait()
                write_cache(k_buf, dk_hbm, 0)
                tail_read.wait()

            attn, dxn = carry
            k_ref, v_ref = k_buf.at[h], v_buf.at[h]
            cols = _block(h, head_dim)
            q = _matmul(xn, wq_buf[:, cols])
            do = _matmul_t(d_attn, wo_buf[cols, :])
            s = _matmul_t(q, k_ref[...]) * scale
            dp = _matmul_t(do, v_ref[...])
            e = jnp.exp(s - jnp.max(s, axis=-1, keepdims=True))
            p = e * (1.0 / jnp.sum(e, axis=-1, keepdims=True))
            ds = p * (dp - jnp.sum(p * dp, axis=-1, keepdims=True)) * scale
            o = _matmul(p, v_ref[...])
            dq = _matmul(ds, k_ref[...])
            attn += _matmul(o, wo_buf[cols, :])
            dxn += _matmul_t(dq, wq_buf[:, cols])
            _store_tall_outer(v_ref, p, do)
            _store_tall_outer(k_ref, ds, q)
            wq_buf[:, cols] = (xn_col[...] * dq[0:1]).astype(BF16)
            _store_outer(wo_buf.at[cols], o, d_attn)
            return attn, dxn

        zero = jnp.zeros((SUBLANES, d_model), F32)
        attn, dxn = lax.fori_loop(0, heads, head, (zero, zero))

        write_cache(v_buf, dv_hbm, 0)
        df = dy * attn * (sig + gate * (1.0 - sig))
        dmid = _matmul_t(df, wd_buf[...])
        inner_slope = GELU_C * (1.0 + 3.0 * GELU_A * a * a)
        dact = 0.5 * (1.0 + t) + 0.5 * a * (1.0 - t * t) * inner_slope
        da = dmid * u * dact
        du = dmid * act
        dxn = dxn + _matmul(da, wg_buf[...]) + _matmul(du, wu_buf[...])
        dx = dy + rstd * (dxn - _mean(dxn) - xn * _mean(dxn * xn))
        x_buf[0] = (x + attn * gate)[0:1].astype(BF16)
        dy_buf[0] = dx[0:1].astype(BF16)

        write_cache(k_buf, dk_hbm, 1)
        _store_outer(wg_buf, da, xn)
        _store_outer(wu_buf, du, xn)
        _store_outer(wd_buf, mid, df)
        write_cache(v_buf, dv_hbm, 1)

    pl.run_scoped(
        read_and_compute,
        pltpu.SemaphoreType.DMA((heads,)),
        pltpu.SemaphoreType.DMA((3,)),
    )

    ffn_grads = [(wg_buf, dwg_hbm), (wu_buf, dwu_hbm), (wd_buf, dwd_hbm)]
    copy(x_buf, y_hbm, write_sem).start()
    copy(dy_buf, dx_hbm, write_sem).start()
    write_weights([(wq_buf, dwq_hbm)], regions=8, rows=8, cols=256)
    write_weights([(wo_buf, dwo_hbm)], regions=4, rows=8, cols=d_model)
    write_weights(ffn_grads, regions=2, rows=16, cols=d_model)
    for group in range(2, heads // WRITE_HEADS):
        write_cache(k_buf, dk_hbm, group)
        write_cache(v_buf, dv_hbm, group)

    written = [
        (x_buf, y_hbm), (dy_buf, dx_hbm), (wq_buf, dwq_hbm), (wo_buf, dwo_hbm),
        *ffn_grads, (k_buf, dk_hbm.at[0]), (v_buf, dv_hbm.at[0]),
    ]
    for buf, hbm in written:
        copy(buf, hbm, write_sem).wait()


@jax.jit
def pallas_recurrent_scan__gqa_block_cached__geglu_ffn__decode_kernel(
    A_x: jax.Array,
    A_k_cache: jax.Array,
    A_v_cache: jax.Array,
    A_wq: jax.Array,
    A_wo: jax.Array,
    B_x: jax.Array,
    B_w_gate: jax.Array,
    B_w_up: jax.Array,
    B_w_down: jax.Array,
    grad_out: jax.Array,
):
    del B_x
    w_gate_t, w_up_t = B_w_gate.T, B_w_up.T
    weights = (A_wq, A_wo, w_gate_t, w_up_t, B_w_down)
    operands = (A_x, A_k_cache, A_v_cache, *weights, grad_out)
    results = (A_x, A_x, A_k_cache, A_v_cache, *weights)
    hbm = pl.BlockSpec(memory_space=pltpu.HBM)

    y, dx, dk, dv, dwq, dwo, dw_gate_t, dw_up_t, dw_down = pl.pallas_call(
        _kernel,
        in_specs=[hbm] * len(operands),
        out_specs=[hbm] * len(results),
        out_shape=[jax.ShapeDtypeStruct(r.shape, BF16) for r in results],
        scratch_shapes=[
            pltpu.VMEM(A_x.shape, BF16),
            pltpu.VMEM(grad_out.shape, BF16),
            pltpu.VMEM(A_k_cache.shape[1:], BF16),
            pltpu.VMEM(A_v_cache.shape[1:], BF16),
            *[pltpu.VMEM(w.shape, BF16) for w in weights],
            pltpu.VMEM((A_x.shape[-1], LANES), F32),
            pltpu.SemaphoreType.DMA,
        ],
        compiler_params=pltpu.CompilerParams(vmem_limit_bytes=100 * 1024 * 1024),
    )(*operands)
    return y, dx, dk, dv, dwq, dwo, dw_gate_t.T, dw_up_t.T, dw_down
```

```python
import math

import jax
import jax.numpy as jnp
from jax import lax
import jax.experimental.pallas as pl
import jax.experimental.pallas.tpu as pltpu

F32 = jnp.float32
BF16 = jnp.bfloat16
LANES = 128
SUBLANES = 8
LN_EPS = 1e-5
GELU_C = math.sqrt(2.0 / math.pi)
GELU_A = 0.044715

WRITE_HEAD_GROUPS = (7, 7, 6, 6, 6)
WRITE_ROWS = 16
READ_TAIL_ROWS = 1792


def _matmul(a, b):
    return jnp.dot(a.astype(BF16), b, preferred_element_type=F32)


def _matmul_t(a, b):
    return lax.dot_general(
        a.astype(BF16), b, (((1,), (1,)), ((), ())), preferred_element_type=F32
    )


def _mean(v):
    return jnp.mean(v, axis=-1, keepdims=True)


def _block(index, size):
    return pl.ds(pl.multiple_of(index * size, size), size)


def _column(row):
    return jnp.broadcast_to(row, (LANES, LANES)).T


def _store_outer(out_ref, left, right):
    n = left.shape[1]
    for i in range(0, n, LANES):
        i = min(i, n - LANES)
        col = _column(left[0:1, i:i + LANES])
        for j in range(0, right.shape[1], LANES):
            tile = col * right[0:1, j:j + LANES]
            out_ref[i:i + LANES, j:j + LANES] = tile.astype(out_ref.dtype)


def _store_tall_outer(out_ref, left, right):
    col = _column(right[0:1])
    for i in range(0, left.shape[1], LANES):
        tile = col * left[0:1, i:i + LANES]
        out_ref[i:i + LANES, :] = tile.astype(out_ref.dtype).T


def _kernel(
    x_hbm, k_hbm, v_hbm, wq_hbm, wo_hbm, wg_hbm, wu_hbm, wd_hbm, dy_hbm,
    y_hbm, dx_hbm, dk_hbm, dv_hbm, dwq_hbm, dwo_hbm, dwg_hbm, dwu_hbm, dwd_hbm,
    x_buf, dy_buf, k_buf, v_buf, wq_buf, wo_buf, wg_buf, wu_buf, wd_buf,
    xn_col, write_sem,
):
    heads, seq, head_dim = k_buf.shape
    d_model = x_buf.shape[-1]
    scale = head_dim ** -0.5
    last = heads - 1
    copy = pltpu.make_async_copy

    assert sum(WRITE_HEAD_GROUPS) == heads

    def write_cache(buf, hbm, group):
        hs = pl.ds(sum(WRITE_HEAD_GROUPS[:group]), WRITE_HEAD_GROUPS[group])

        @pl.loop(0, seq // WRITE_ROWS, unroll=4)
        def _(j):
            rows = _block(j, WRITE_ROWS)
            copy(buf.at[hs, rows], hbm.at[0, hs, rows], write_sem).start()

    def write_weights(pairs, regions, rows, cols):
        views = []
        for buf, hbm in pairs:
            n_rows, n_cols = buf.shape
            shape = (regions, n_rows // regions, n_cols)
            views.append((buf.reshape(shape), hbm.reshape(shape), n_cols // cols))
        blocks = math.prod(pairs[0][0].shape) // (regions * rows * cols)
        per_step = max(per_row for _, _, per_row in views)

        @pl.loop(0, blocks // per_step)
        def _(j):
            for i in range(per_step):
                for src, dst, per_row in views:
                    row = j * (per_step // per_row) + i // per_row
                    col = i % per_row * cols
                    idx = (slice(None), _block(row, rows), pl.ds(col, cols))
                    copy(src.at[idx], dst.at[idx], write_sem).start()

    def read_and_compute(head_sems, sems):
        ffn_reads = [
            copy(hbm, buf, sems.at[0])
            for hbm, buf in (
                (wg_hbm, wg_buf), (x_hbm, x_buf), (dy_hbm, dy_buf),
                (wu_hbm, wu_buf), (wd_hbm, wd_buf),
            )
        ]
        projection_reads = [
            copy(wq_hbm, wq_buf, sems.at[1]),
            copy(wo_hbm, wo_buf, sems.at[1]),
        ]
        body = pl.ds(0, seq - READ_TAIL_ROWS)
        tail = pl.ds(seq - READ_TAIL_ROWS, READ_TAIL_ROWS)
        tail_read = copy(v_hbm.at[0, last, tail], v_buf.at[last, tail], sems.at[2])

        def k_read(h):
            return copy(k_hbm.at[0, h], k_buf.at[h], head_sems.at[h])

        def v_read(h, rows=slice(None)):
            return copy(v_hbm.at[0, h, rows], v_buf.at[h, rows], head_sems.at[h])

        for c in ffn_reads + projection_reads:
            c.start()

        @pl.loop(0, last)
        def _(h):
            k_read(h).start()
            v_read(h).start()

        k_read(last).start()
        v_read(last, body).start()
        tail_read.start()

        for c in ffn_reads:
            c.wait()
        x = jnp.broadcast_to(x_buf[0].astype(F32), (SUBLANES, d_model))
        dy = jnp.broadcast_to(dy_buf[0].astype(F32), (SUBLANES, d_model))
        centred = x - _mean(x)
        rstd = lax.rsqrt(_mean(centred * centred) + LN_EPS)
        xn = centred * rstd
        for i in range(0, d_model, LANES):
            xn_col[i:i + LANES, :] = _column(xn[0:1, i:i + LANES])

        a = _matmul_t(xn, wg_buf[...])
        u = _matmul_t(xn, wu_buf[...])
        t = jnp.tanh(GELU_C * (a + GELU_A * a * a * a))
        act = 0.5 * a * (1.0 + t)
        mid = act * u
        f = _matmul(mid, wd_buf[...])
        sig = jax.nn.sigmoid(f)
        gate = f * sig
        d_attn = dy * gate

        for c in projection_reads:
            c.wait()

        def head(h, carry):
            k_read(h).wait()

            @pl.when(h < last)
            def _():
                v_read(h).wait()

            @pl.when(h == last)
            def _():
                v_read(last, body).wait()
                write_cache(k_buf, dk_hbm, 0)
                tail_read.wait()

            attn, dxn = carry
            k_ref, v_ref = k_buf.at[h], v_buf.at[h]
            cols = _block(h, head_dim)
            q = _matmul(xn, wq_buf[:, cols])
            do = _matmul_t(d_attn, wo_buf[cols, :])
            s = _matmul_t(q, k_ref[...]) * scale
            dp = _matmul_t(do, v_ref[...])
            e = jnp.exp(s - jnp.max(s, axis=-1, keepdims=True))
            p = e * (1.0 / jnp.sum(e, axis=-1, keepdims=True))
            ds = p * (dp - jnp.sum(p * dp, axis=-1, keepdims=True)) * scale
            o = _matmul(p, v_ref[...])
            dq = _matmul(ds, k_ref[...])
            attn += _matmul(o, wo_buf[cols, :])
            dxn += _matmul_t(dq, wq_buf[:, cols])
            _store_tall_outer(v_ref, p, do)
            _store_tall_outer(k_ref, ds, q)
            wq_buf[:, cols] = (xn_col[...] * dq[0:1]).astype(BF16)
            _store_outer(wo_buf.at[cols], o, d_attn)
            return attn, dxn

        zero = jnp.zeros((SUBLANES, d_model), F32)
        attn, dxn = lax.fori_loop(0, heads, head, (zero, zero))

        write_cache(v_buf, dv_hbm, 0)
        df = dy * attn * (sig + gate * (1.0 - sig))
        dmid = _matmul_t(df, wd_buf[...])
        inner_slope = GELU_C * (1.0 + 3.0 * GELU_A * a * a)
        dact = 0.5 * (1.0 + t) + 0.5 * a * (1.0 - t * t) * inner_slope
        da = dmid * u * dact
        du = dmid * act
        dxn = dxn + _matmul(da, wg_buf[...]) + _matmul(du, wu_buf[...])
        dx = dy + rstd * (dxn - _mean(dxn) - xn * _mean(dxn * xn))
        x_buf[0] = (x + attn * gate)[0:1].astype(BF16)
        dy_buf[0] = dx[0:1].astype(BF16)

        write_cache(k_buf, dk_hbm, 1)
        _store_outer(wg_buf, da, xn)
        _store_outer(wu_buf, du, xn)
        _store_outer(wd_buf, mid, df)
        write_cache(v_buf, dv_hbm, 1)

    pl.run_scoped(
        read_and_compute,
        pltpu.SemaphoreType.DMA((heads,)),
        pltpu.SemaphoreType.DMA((3,)),
    )

    projection_grads = [(wq_buf, dwq_hbm), (wo_buf, dwo_hbm)]
    ffn_grads = [(wg_buf, dwg_hbm), (wu_buf, dwu_hbm), (wd_buf, dwd_hbm)]
    copy(x_buf, y_hbm, write_sem).start()
    copy(dy_buf, dx_hbm, write_sem).start()
    for group in range(2, len(WRITE_HEAD_GROUPS)):
        write_cache(k_buf, dk_hbm, group)
        write_cache(v_buf, dv_hbm, group)
    write_weights(ffn_grads, regions=2, rows=16, cols=d_model)
    write_weights(projection_grads, regions=4, rows=8, cols=256)

    written = [
        (x_buf, y_hbm), (dy_buf, dx_hbm), *projection_grads, *ffn_grads,
        (k_buf, dk_hbm.at[0]), (v_buf, dv_hbm.at[0]),
    ]
    for buf, hbm in written:
        copy(buf, hbm, write_sem).wait()


@jax.jit
def pallas_recurrent_scan__gqa_block_cached__geglu_ffn__decode_kernel(
    A_x: jax.Array,
    A_k_cache: jax.Array,
    A_v_cache: jax.Array,
    A_wq: jax.Array,
    A_wo: jax.Array,
    B_x: jax.Array,
    B_w_gate: jax.Array,
    B_w_up: jax.Array,
    B_w_down: jax.Array,
    grad_out: jax.Array,
):
    del B_x
    w_gate_t, w_up_t = B_w_gate.T, B_w_up.T
    weights = (A_wq, A_wo, w_gate_t, w_up_t, B_w_down)
    operands = (A_x, A_k_cache, A_v_cache, *weights, grad_out)
    results = (A_x, A_x, A_k_cache, A_v_cache, *weights)
    hbm = pl.BlockSpec(memory_space=pltpu.HBM)

    y, dx, dk, dv, dwq, dwo, dw_gate_t, dw_up_t, dw_down = pl.pallas_call(
        _kernel,
        in_specs=[hbm] * len(operands),
        out_specs=[hbm] * len(results),
        out_shape=[jax.ShapeDtypeStruct(r.shape, BF16) for r in results],
        scratch_shapes=[
            pltpu.VMEM(A_x.shape, BF16),
            pltpu.VMEM(grad_out.shape, BF16),
            pltpu.VMEM(A_k_cache.shape[1:], BF16),
            pltpu.VMEM(A_v_cache.shape[1:], BF16),
            *[pltpu.VMEM(w.shape, BF16) for w in weights],
            pltpu.VMEM((A_x.shape[-1], LANES), F32),
            pltpu.SemaphoreType.DMA,
        ],
        compiler_params=pltpu.CompilerParams(vmem_limit_bytes=100 * 1024 * 1024),
    )(*operands)
    return y, dx, dk, dv, dwq, dwo, dw_gate_t.T, dw_up_t.T, dw_down
```
